```python
import jax
import jax.numpy as jnp

def _softmax(x, axis=-1):
    return jax.nn.softmax(x, axis=axis)
def _gelu(x):
    return jax.nn.gelu(x, approximate=True)
def _silu(x):
    return jax.nn.silu(x)
def _sigmoid(x):
    return jax.nn.sigmoid(x)
def _layernorm(x, axis=-1, eps=1e-5):
    m = jnp.mean(x, axis=axis, keepdims=True)
    v = jnp.var(x, axis=axis, keepdims=True)
    return (x - m) / jnp.sqrt(v + eps)
def _scatter_add(tgt, idx, src, axis=0):
    return tgt.at[idx].add(src)
def _segment_sum(src, seg, n):
    return jax.ops.segment_sum(src, seg, n)
class _Rng:
    def __init__(self, key):
        self._k = key
    def _next(self):
        self._k, sub = jax.random.split(self._k)
        return sub
    def normal(self, shape):
        return jax.random.normal(self._next(), shape, dtype=jnp.bfloat16)
    def randint(self, lo, hi, shape):
        return jax.random.randint(self._next(), shape, lo, hi, dtype=jnp.int32)
    def uniform(self, shape, lo=0.0, hi=1.0):
        return jax.random.uniform(self._next(), shape, jnp.bfloat16, lo, hi)
    def permutation(self, n):
        return jax.random.permutation(self._next(), n)


kernel_name = 'recurrent_scan__sliding_local_dilated__glu_gated_swiglu__prompt'

def setup_inputs():
    _rng = _Rng(jax.random.key(int.from_bytes(__import__("os").urandom(4), "little")))
    _w = (lambda a: (lambda t: t.astype(jnp.bfloat16) if jnp.issubdtype(t.dtype, jnp.floating) else t)(jnp.asarray(a)))
    def _A_setup():
        B, S, D = 1, 2048, 1024
        return {
            "x": _w((lambda *s: _rng.normal(s) * 0.05)(B, S, D)),
            "wqkv": _w((lambda *s: _rng.normal(s) * 0.05)(D, 3 * D)),
            "wo": _w((lambda *s: _rng.normal(s) * 0.05)(D, D)),
        }
    _A_in = _A_setup()

    def _B_setup():
        B, S, D, F = 1, 2048, 1024, 3584
        return {
            "x": _w((lambda *s: _rng.normal(s) * 0.05)(B, S, D)),
            "w1": _w((lambda *s: _rng.normal(s) * 0.05)(D, F) * (2.0 / D) ** 0.5),
            "w3": _w((lambda *s: _rng.normal(s) * 0.05)(D, F) * (2.0 / D) ** 0.5),
            "w2": _w((lambda *s: _rng.normal(s) * 0.05)(F, D) * (2.0 / F) ** 0.5),
        }
    _B_in = _B_setup()

    return {
        "A_x": _A_in["x"],
        "A_wqkv": _A_in["wqkv"],
        "A_wo": _A_in["wo"],
        "B_x": _B_in["x"],
        "B_w1": _B_in["w1"],
        "B_w3": _B_in["w3"],
        "B_w2": _B_in["w2"],
    }

def reference(A_x, A_wqkv, A_wo, B_x, B_w1, B_w3, B_w2):
    def _A_ref(x, wqkv, wo):
        B, S, D = x.shape
        H = 32; Dh = D // H
        W, dil = 8, 2
        qkv = (lambda x, *d: x.transpose(*d))((x @ wqkv).reshape(B, S, 3, H, Dh), 2, 0, 3, 1, 4)
        q, k, v = qkv[0], qkv[1], qkv[2]
        scale = Dh ** -0.5
        pos = jnp.arange(S)
        off = jnp.arange(W) * dil
        idx = pos[:, None] - off[None, :]
        mask = idx >= 0
        idx_c = jnp.where(mask, idx, 0).reshape(-1)
        kg = k[:, :, idx_c, :].reshape(B, H, S, W, Dh)
        vg = v[:, :, idx_c, :].reshape(B, H, S, W, Dh)
        logits = jnp.einsum("bhsd,bhswd->bhsw", q, kg) * scale
        logits = jnp.where(mask[None, None, :, :], logits, -1e9)
        attn = _softmax(logits, axis=-1)
        o = jnp.einsum("bhsw,bhswd->bhsd", attn, vg)
        return (lambda x, *d: x.transpose(*d))(o, 0, 2, 1, 3).reshape(B, S, D) @ wo

    def _B_ref(x, w1, w3, w2):
        gate = jnp.einsum("bsd,df->bsf", x, w1)
        up = jnp.einsum("bsd,df->bsf", x, w3)
        h = _silu(gate) * up
        out = jnp.einsum("bsf,fd->bsd", h, w2)
        return out

    x = A_x
    xn = _layernorm(x, axis=-1)
    s = _A_ref(xn, A_wqkv, A_wo)
    g = _silu(_B_ref(xn, B_w1, B_w3, B_w2))
    return x + s * g
```

```python
import functools

import jax
import jax.numpy as jnp
from jax.experimental import pallas as pl
from jax.experimental.pallas import tpu as pltpu

S = 2048
D = 1024
F = 3584
H = 32
DH = D // H
W = 8
DIL = 2
PAD = 16
LANES = 128
NT = D // LANES
TA = 128
TP = 256
TB = 256
FC = 512
QC = 512
RA = 32
NXB = S // TA + 1
EPS = 1e-5
MASK_VALUE = -1e9

f32 = jnp.float32
bf16 = jnp.bfloat16


def _butterfly(tiles, lane):
    t = list(tiles)
    for b in range(3):
        s = 4 << b
        m = (lane & s) != 0
        nt = list(t)
        for a in range(NT):
            if a & (1 << b):
                continue
            c = a | (1 << b)
            nt[a] = jnp.where(m, pltpu.roll(t[c], s, 1), t[a])
            nt[c] = jnp.where(m, t[c], pltpu.roll(t[a], LANES - s, 1))
        t = nt
    return t


def _layernorm(x):
    x = x.astype(f32)
    m = jnp.mean(x, axis=-1, keepdims=True)
    xc = x - m
    v = jnp.mean(xc * xc, axis=-1, keepdims=True)
    return (xc * jax.lax.rsqrt(v + EPS)).astype(bf16)


def _kernel(x_hbm, wqkv_hbm, wo_hbm, w1_hbm, w3_hbm, w2_hbm, out_hbm,
            x_v, xn_v, wqkv_v, wo_v, w1_v, w3_v, w2_v, qkv_v, o_v, out_v,
            x_sem, wq_sem, w_sem, out_sem):

    def x_copy(b):
        src = min(b, S // TA - 1)
        return pltpu.make_async_copy(
            x_hbm.at[pl.ds(src * TA, TA)], x_v.at[pl.ds(b * TA, TA)], x_sem.at[b])

    def x_wait(b):
        start = pl.multiple_of(b * TA, TA)
        pltpu.make_async_copy(
            x_hbm.at[pl.ds(0, TA)], x_v.at[pl.ds(start, TA)], x_sem.at[b]).wait()

    def wq_copy(c):
        return pltpu.make_async_copy(
            wqkv_hbm.at[:, pl.ds(c * QC, QC)], wqkv_v.at[:, pl.ds(c * QC, QC)], wq_sem.at[c])

    w_copies = [
        pltpu.make_async_copy(w1_hbm, w1_v, w_sem.at[0]),
        pltpu.make_async_copy(w3_hbm, w3_v, w_sem.at[1]),
        pltpu.make_async_copy(w2_hbm, w2_v, w_sem.at[2]),
        pltpu.make_async_copy(wo_hbm, wo_v, w_sem.at[3]),
    ]

    def out_copy(i):
        start = i * TB if isinstance(i, int) else pl.multiple_of(i * TB, TB)
        return pltpu.make_async_copy(
            out_v.at[pl.ds(start, TB)], out_hbm.at[pl.ds(start, TB)], out_sem.at[i])

    nq = 3 * D // QC
    x_copy(0).start()
    x_copy(1).start()
    for c in range(nq):
        wq_copy(c).start()
    for b in range(2, NXB):
        x_copy(b).start()

    qkv_v[:, 0:PAD, :] = jnp.zeros((3 * NT, PAD, LANES), f32)

    def do_ln(start, rows):
        for r in range(0, rows, 32):
            xn_v[pl.ds(start + r, 32), :] = _layernorm(x_v[pl.ds(start + r, 32), :])

    def do_qkv(start, rows, wait_w):
        lane = jax.lax.broadcasted_iota(jnp.int32, (rows, LANES), 1)
        for sec in range(3):
            parts = []
            for c in range(sec * (D // QC), (sec + 1) * (D // QC)):
                if wait_w:
                    wq_copy(c).wait()
                parts.append(jnp.dot(xn_v[pl.ds(start, rows), :], wqkv_v[:, c * QC:(c + 1) * QC],
                                     preferred_element_type=f32))
            tiles = []
            for p in parts:
                tiles += [p[:, j * LANES:(j + 1) * LANES] for j in range(QC // LANES)]
            tiles = _butterfly(tiles, lane)
            for j in range(NT):
                qkv_v[sec * NT + j, pl.ds(PAD + start, rows), :] = tiles[j]

    x_copy(0).wait()
    x_copy(1).wait()
    do_ln(0, TP)
    do_qkv(0, TP, True)
    x_copy(2).wait()
    do_ln(TP, TA)
    for cp in w_copies:
        cp.start()

    def body_a(i, carry):
        x_wait(i + 1)
        start = pl.multiple_of(i * TA, TA)
        do_qkv(start, TA, False)
        do_ln(start + TA, TA)
        return carry

    jax.lax.fori_loop(TP // TA, S // TA, body_a, 0)

    for cp in w_copies:
        cp.wait()

    def attention(base, r):
        lane = jax.lax.broadcasted_iota(jnp.int32, (RA, LANES), 1)
        row = jax.lax.broadcasted_iota(jnp.int32, (RA, LANES), 0)
        m1 = (lane & 1) != 0
        m2 = (lane & 2) != 0
        start = base + (PAD + r)
        tok = row + (base + r)
        q = [qkv_v[j, pl.ds(start, RA), :] for j in range(NT)]
        ls = []
        for w in range(W):
            acc = None
            for j in range(NT):
                p = q[j] * qkv_v[NT + j, pl.ds(start - DIL * w, RA), :]
                acc = p if acc is None else acc + p
            acc = acc + jnp.where(m1, pltpu.roll(acc, 1, 1), pltpu.roll(acc, LANES - 1, 1))
            acc = acc + jnp.where(m2, pltpu.roll(acc, 2, 1), pltpu.roll(acc, LANES - 2, 1))
            acc = acc * (DH ** -0.5)
            if w > 0:
                acc = jnp.where(tok >= DIL * w, acc, MASK_VALUE)
            ls.append(acc)
        mx = functools.reduce(jnp.maximum, ls)
        es = [jnp.exp(l - mx) for l in ls]
        inv = 1.0 / functools.reduce(lambda a, b: a + b, es)
        ps = [e * inv for e in es]
        o = []
        for j in range(NT):
            acc = None
            for w in range(W):
                p = ps[w] * qkv_v[2 * NT + j, pl.ds(start - DIL * w, RA), :]
                acc = p if acc is None else acc + p
            o.append(acc)
        o = _butterfly(o, lane)
        o_v[pl.ds(r, RA), :] = jnp.concatenate(o, axis=1).astype(bf16)

    def body_b(i, carry):
        base = pl.multiple_of(i * TB, TB)
        rows = pl.ds(base, TB)
        nc = F // FC
        pieces = list(range(0, TB, RA))
        acc = None
        for c in range(nc):
            sl = slice(c * FC, (c + 1) * FC)
            g = jnp.dot(xn_v[rows, :], w1_v[:, sl], preferred_element_type=f32)
            u = jnp.dot(xn_v[rows, :], w3_v[:, sl], preferred_element_type=f32)
            h = (g * jax.nn.sigmoid(g) * u).astype(bf16)
            d = jnp.dot(h, w2_v[sl, :], preferred_element_type=f32)
            acc = d if acc is None else acc + d
            lo = (len(pieces) * c) // (nc - 1) if c < nc - 1 else len(pieces)
            hi = (len(pieces) * (c + 1)) // (nc - 1) if c < nc - 1 else len(pieces)
            for r in pieces[lo:hi]:
                attention(base, r)
        s = jnp.dot(o_v[...], wo_v[...], preferred_element_type=f32)
        gate = acc * jax.nn.sigmoid(acc)
        out_v[rows, :] = (x_v[rows, :].astype(f32) + s * gate).astype(bf16)
        out_copy(i).start()
        return carry

    jax.lax.fori_loop(0, S // TB, body_b, 0)
    for i in range(S // TB):
        out_copy(i).wait()


@jax.jit
def pallas_recurrent_scan__sliding_local_dilated__glu_gated_swiglu__prompt_kernel(
    A_x: jax.Array,
    A_wqkv: jax.Array,
    A_wo: jax.Array,
    B_x: jax.Array,
    B_w1: jax.Array,
    B_w3: jax.Array,
    B_w2: jax.Array,
):
    x = A_x.reshape(S, D)
    any_spec = pl.BlockSpec(memory_space=pl.ANY)
    out = pl.pallas_call(
        _kernel,
        out_shape=jax.ShapeDtypeStruct((S, D), bf16),
        in_specs=[any_spec] * 6,
        out_specs=any_spec,
        scratch_shapes=[
            pltpu.VMEM((S + TA, D), bf16),
            pltpu.VMEM((S + TA, D), bf16),
            pltpu.VMEM((D, 3 * D), bf16),
            pltpu.VMEM((D, D), bf16),
            pltpu.VMEM((D, F), bf16),
            pltpu.VMEM((D, F), bf16),
            pltpu.VMEM((F, D), bf16),
            pltpu.VMEM((3 * NT, PAD + S, LANES), f32),
            pltpu.VMEM((TB, D), bf16),
            pltpu.VMEM((S, D), bf16),
            pltpu.SemaphoreType.DMA((NXB,)),
            pltpu.SemaphoreType.DMA((3 * D // QC,)),
            pltpu.SemaphoreType.DMA((4,)),
            pltpu.SemaphoreType.DMA((S // TB,)),
        ],
        compiler_params=pltpu.CompilerParams(vmem_limit_bytes=120 * 1024 * 1024),
    )(x, A_wqkv, A_wo, B_w1, B_w3, B_w2)
    return out.reshape(1, S, D)
```

```python
import functools

import jax
import jax.numpy as jnp
from jax.experimental import pallas as pl
from jax.experimental.pallas import tpu as pltpu

S = 2048
D = 1024
F = 3584
H = 32
DH = D // H
W = 8
DIL = 2
PAD = 16
LANES = 128
NT = D // LANES
TA = 256
TB = 256
NB = S // TB
FC = 512
WS = D // NB
RA = 16
RP = 40
EPS = 1e-5
MASK_VALUE = -1e9

f32 = jnp.float32
bf16 = jnp.bfloat16


def _swap_tile_lane_bits(tiles):
    lane = jax.lax.broadcasted_iota(jnp.int32, tiles[0].shape, 1)
    r = [tiles[0]] + [pltpu.roll(tiles[t], 4 * t, 1) for t in range(1, NT)]
    u = [r[(-k) % NT] for k in range(NT)]
    for b in range(3):
        m = (lane & (4 << b)) != 0
        u = [jnp.where(m, u[(k - (1 << b)) % NT], u[k]) for k in range(NT)]
    return [u[0]] + [pltpu.roll(u[t], LANES - 4 * t, 1) for t in range(1, NT)]


def _layernorm(x):
    x = x.astype(f32)
    m = jnp.mean(x, axis=-1, keepdims=True)
    xc = x - m
    v = jnp.mean(xc * xc, axis=-1, keepdims=True)
    return (xc * jax.lax.rsqrt(v + EPS)).astype(bf16)


def _kernel(x_hbm, wqkv_hbm, wo_hbm, w1_hbm, w3_hbm, w2_hbm, out_hbm,
            x_v, xn_v, wq_v, wk_v, wv_v, wo_v, w1_v, w3_v, w2_v,
            q_v, k_v, v_v, o_v, out_v,
            x_sem, wq_sem, wk_sem, wv_sem, w_sem, out_sem):

    def blk(i, n):
        return i * n if isinstance(i, int) else pl.multiple_of(i * n, n)

    def x_copy(b):
        src = min(b, NB - 1) if isinstance(b, int) else 0
        return pltpu.make_async_copy(
            x_hbm.at[pl.ds(src * TA, TA)], x_v.at[pl.ds(blk(b, TA), TA)], x_sem.at[b])

    def w_slice_copy(sec, dst, sem, s):
        rows = pl.ds(blk(s, WS), WS)
        return pltpu.make_async_copy(
            wqkv_hbm.at[rows, pl.ds(sec * D, D)], dst.at[rows], sem.at[s])

    wq_copy = functools.partial(w_slice_copy, 0, wq_v, wq_sem)
    wk_copy = functools.partial(w_slice_copy, 1, wk_v, wk_sem)
    wv_copy = functools.partial(w_slice_copy, 2, wv_v, wv_sem)

    w_copies = [
        pltpu.make_async_copy(w1_hbm, w1_v, w_sem.at[0]),
        pltpu.make_async_copy(w3_hbm, w3_v, w_sem.at[1]),
        pltpu.make_async_copy(w2_hbm, w2_v, w_sem.at[2]),
        pltpu.make_async_copy(wo_hbm, wo_v, w_sem.at[3]),
    ]

    def out_copy(i):
        rows = pl.ds(blk(i, TB), TB)
        return pltpu.make_async_copy(out_v.at[rows], out_hbm.at[rows], out_sem.at[i])

    def permute_weight(w_ref, s):
        rows = pl.ds(blk(s, WS), WS)
        tiles = [pltpu.bitcast(w_ref[rows, j * LANES:(j + 1) * LANES], jnp.uint32)
                 for j in range(NT)]
        tiles = _swap_tile_lane_bits(tiles)
        for j in range(NT):
            w_ref[rows, j * LANES:(j + 1) * LANES] = pltpu.bitcast(tiles[j], bf16)

    def do_ln(start):
        for r in range(0, TA, 32):
            xn_v[pl.ds(start + r, 32), :] = _layernorm(x_v[pl.ds(start + r, 32), :])

    def project(w_ref, dst, start, scale=None):
        res = jnp.dot(xn_v[pl.ds(start, TA), :], w_ref[...], preferred_element_type=f32)
        if scale is not None:
            res = res * scale
        for j in range(NT):
            dst[j, pl.ds(PAD + start, TA), :] = res[:, j * LANES:(j + 1) * LANES]

    def attention(tok0, rows, masked, store):
        lane = jax.lax.broadcasted_iota(jnp.int32, (rows, LANES), 1)
        m1 = (lane & 1) != 0
        m2 = (lane & 2) != 0
        start = tok0 + PAD
        q = [q_v[j, pl.ds(start, rows), :] for j in range(NT)]
        ls = []
        for w in range(W):
            acc = None
            for j in range(NT):
                p = q[j] * k_v[j, pl.ds(start - DIL * w, rows), :]
                acc = p if acc is None else acc + p
            acc = acc + jnp.where(m1, pltpu.roll(acc, 1, 1), pltpu.roll(acc, LANES - 1, 1))
            acc = acc + jnp.where(m2, pltpu.roll(acc, 2, 1), pltpu.roll(acc, LANES - 2, 1))
            if masked and w > 0:
                tok = jax.lax.broadcasted_iota(jnp.int32, (rows, LANES), 0) + tok0
                acc = jnp.where(tok >= DIL * w, acc, MASK_VALUE)
            ls.append(acc)
        mx = functools.reduce(jnp.maximum, ls)
        es = [jnp.exp(l - mx) for l in ls]
        inv = 1.0 / functools.reduce(lambda a, b: a + b, es)
        ps = [e * inv for e in es]
        o = []
        for j in range(NT):
            acc = None
            for w in range(W):
                p = ps[w] * v_v[j, pl.ds(start - DIL * w, rows), :]
                acc = p if acc is None else acc + p
            o.append(acc)
        o = _swap_tile_lane_bits(o)
        store(jnp.concatenate(o, axis=1).astype(bf16))

    x_copy(0).start()
    for s in range(NB):
        wk_copy(s).start()
    x_copy(1).start()
    wv_copy(0).start()

    zeros = jnp.zeros((NT, PAD, LANES), f32)
    k_v[:, 0:PAD, :] = zeros
    v_v[:, 0:PAD, :] = zeros

    x_copy(0).wait()
    do_ln(0)
    for s in range(NB):
        wk_copy(s).wait()
        permute_weight(wk_v, s)
    for s in range(1, NB):
        x_copy(s + 1).start()
        wv_copy(s).start()
    for s in range(NB):
        wq_copy(s).start()

    def body_k(i, carry):
        x_copy(i + 1).wait()
        wv_copy(i).wait()
        start = blk(i, TA)
        project(wk_v, k_v, start)
        do_ln(start + TA)
        permute_weight(wv_v, i)
        return carry

    jax.lax.fori_loop(0, NB, body_k, 0)
    for cp in w_copies:
        cp.start()

    def body_v(i, carry):
        wq_copy(i).wait()
        project(wv_v, v_v, blk(i, TA))
        permute_weight(wq_v, i)
        return carry

    jax.lax.fori_loop(0, NB, body_v, 0)

    def body_q(i, carry):
        tok0 = pl.multiple_of(jnp.clip((i - 1) * RP, 0, TB - RP), 8)

        def store(o):
            o_v[0, pl.ds(tok0, RP), :] = o

        attention(tok0, RP, True, store)
        project(wq_v, q_v, blk(i, TA), DH ** -0.5)
        return carry

    jax.lax.fori_loop(0, NB, body_q, 0)

    for cp in w_copies:
        cp.wait()

    def body_b(i, carry):
        base = blk(i, TB)
        rows = pl.ds(base, TB)
        nbase = pl.multiple_of(jnp.minimum(i + 1, NB - 1) * TB, TB)
        nslot = (i + 1) % 2
        s = jnp.dot(o_v[i % 2], wo_v[...], preferred_element_type=f32)
        nc = F // FC
        pieces = list(range(0, TB, RA))
        acc = None
        for c in range(nc):
            sl = slice(c * FC, (c + 1) * FC)
            g = jnp.dot(xn_v[rows, :], w1_v[:, sl], preferred_element_type=f32)
            u = jnp.dot(xn_v[rows, :], w3_v[:, sl], preferred_element_type=f32)
            h = (g * jax.nn.sigmoid(g) * u).astype(bf16)
            d = jnp.dot(h, w2_v[sl, :], preferred_element_type=f32)
            acc = d if acc is None else acc + d
            lo = (len(pieces) * c) // nc
            hi = (len(pieces) * (c + 1)) // nc
            for r in pieces[lo:hi]:
                def store(o, r=r):
                    o_v[nslot, pl.ds(r, RA), :] = o
                attention(nbase + r, RA, False, store)
        gate = acc * jax.nn.sigmoid(acc)
        out_v[rows, :] = (x_v[rows, :].astype(f32) + s * gate).astype(bf16)
        out_copy(i).start()
        return carry

    jax.lax.fori_loop(0, NB, body_b, 0)
    for i in range(NB):
        out_copy(i).wait()


@jax.jit
def pallas_recurrent_scan__sliding_local_dilated__glu_gated_swiglu__prompt_kernel(
    A_x: jax.Array,
    A_wqkv: jax.Array,
    A_wo: jax.Array,
    B_x: jax.Array,
    B_w1: jax.Array,
    B_w3: jax.Array,
    B_w2: jax.Array,
):
    x = A_x.reshape(S, D)
    any_spec = pl.BlockSpec(memory_space=pl.ANY)
    out = pl.pallas_call(
        _kernel,
        out_shape=jax.ShapeDtypeStruct((S, D), bf16),
        in_specs=[any_spec] * 6,
        out_specs=any_spec,
        scratch_shapes=[
            pltpu.VMEM((S + TA, D), bf16),
            pltpu.VMEM((S + TA, D), bf16),
            pltpu.VMEM((D, D), bf16),
            pltpu.VMEM((D, D), bf16),
            pltpu.VMEM((D, D), bf16),
            pltpu.VMEM((D, D), bf16),
            pltpu.VMEM((D, F), bf16),
            pltpu.VMEM((D, F), bf16),
            pltpu.VMEM((F, D), bf16),
            pltpu.VMEM((NT, PAD + S, LANES), f32),
            pltpu.VMEM((NT, PAD + S, LANES), f32),
            pltpu.VMEM((NT, PAD + S, LANES), f32),
            pltpu.VMEM((2, TB, D), bf16),
            pltpu.VMEM((S, D), bf16),
            pltpu.SemaphoreType.DMA((NB + 1,)),
            pltpu.SemaphoreType.DMA((NB,)),
            pltpu.SemaphoreType.DMA((NB,)),
            pltpu.SemaphoreType.DMA((NB,)),
            pltpu.SemaphoreType.DMA((4,)),
            pltpu.SemaphoreType.DMA((NB,)),
        ],
        compiler_params=pltpu.CompilerParams(vmem_limit_bytes=120 * 1024 * 1024),
    )(x, A_wqkv, A_wo, B_w1, B_w3, B_w2)
    return out.reshape(1, S, D)
```

```python
import functools

import jax
import jax.numpy as jnp
from jax.experimental import pallas as pl
from jax.experimental.pallas import tpu as pltpu

S = 2048
D = 1024
F = 3584
H = 32
DH = D // H
W = 8
DIL = 2
PAD = 16
LANES = 128
NT = D // LANES
TA = 256
TB = 256
NB = S // TB
FC = 512
WS = D // NB
KS = 256
NK = D // KS
RA = 16
RP = 40
EPS = 1e-5
MASK_VALUE = -1e9

f32 = jnp.float32
bf16 = jnp.bfloat16


def _swap_tile_lane_bits(tiles):
    lane = jax.lax.broadcasted_iota(jnp.int32, tiles[0].shape, 1)
    r = [tiles[0]] + [pltpu.roll(tiles[t], 4 * t, 1) for t in range(1, NT)]
    u = [r[(-k) % NT] for k in range(NT)]
    for b in range(3):
        m = (lane & (4 << b)) != 0
        u = [jnp.where(m, u[(k - (1 << b)) % NT], u[k]) for k in range(NT)]
    return [u[0]] + [pltpu.roll(u[t], LANES - 4 * t, 1) for t in range(1, NT)]


def _layernorm(x):
    x = x.astype(f32)
    m = jnp.mean(x, axis=-1, keepdims=True)
    xc = x - m
    v = jnp.mean(xc * xc, axis=-1, keepdims=True)
    return (xc * jax.lax.rsqrt(v + EPS)).astype(bf16)


def _silu(x):
    h = 0.5 * x
    return h + h * jnp.tanh(h)


def _kernel(x_hbm, wqkv_hbm, wo_hbm, w1_hbm, w3_hbm, w2_hbm, out_hbm,
            x_v, xn_v, wq_v, wk_v, wv_v, wo_v, w1_v, w3_v, w2_v,
            q_v, k_v, v_v, o_v, oc_v, out_v,
            x_sem, wq_sem, wk_sem, wv_sem, w_sem, out_sem):

    def blk(i, n):
        return i * n if isinstance(i, int) else pl.multiple_of(i * n, n)

    def x_copy(b):
        src = min(b, NB - 1) if isinstance(b, int) else jnp.minimum(b, NB - 1)
        return pltpu.make_async_copy(
            x_hbm.at[pl.ds(blk(src, TA), TA)], x_v.at[pl.ds(blk(b, TA), TA)], x_sem.at[b])

    def w_slice_copy(sec, dst, sem, n, s):
        rows = pl.ds(blk(s, n), n)
        return pltpu.make_async_copy(
            wqkv_hbm.at[rows, pl.ds(sec * D, D)], dst.at[rows], sem.at[s])

    wq_copy = functools.partial(w_slice_copy, 0, wq_v, wq_sem, WS)
    wk_copy = functools.partial(w_slice_copy, 1, wk_v, wk_sem, KS)
    wv_copy = functools.partial(w_slice_copy, 2, wv_v, wv_sem, WS)

    w_copies = [
        pltpu.make_async_copy(w1_hbm, w1_v, w_sem.at[0]),
        pltpu.make_async_copy(w3_hbm, w3_v, w_sem.at[1]),
        pltpu.make_async_copy(w2_hbm, w2_v, w_sem.at[2]),
        pltpu.make_async_copy(wo_hbm, wo_v, w_sem.at[3]),
    ]

    def out_copy(i):
        rows = pl.ds(blk(i, TB), TB)
        return pltpu.make_async_copy(out_v.at[rows], out_hbm.at[rows], out_sem.at[i])

    def permute_weight(w_ref, s, n):
        rows = pl.ds(blk(s, n), n)
        tiles = [pltpu.bitcast(w_ref[rows, j * LANES:(j + 1) * LANES], jnp.uint32)
                 for j in range(NT)]
        tiles = _swap_tile_lane_bits(tiles)
        for j in range(NT):
            w_ref[rows, j * LANES:(j + 1) * LANES] = pltpu.bitcast(tiles[j], bf16)

    def do_ln(start, r0, rows):
        for r in range(r0, r0 + rows, 32):
            xn_v[pl.ds(start + r, 32), :] = _layernorm(x_v[pl.ds(start + r, 32), :])

    def project(w_ref, dst, start, scale=None):
        res = jnp.dot(xn_v[pl.ds(start, TA), :], w_ref[...], preferred_element_type=f32)
        if scale is not None:
            res = res * scale
        for j in range(NT):
            dst[j, pl.ds(PAD + start, TA), :] = res[:, j * LANES:(j + 1) * LANES]

    def attention(tok0, rows, masked, store):
        lane = jax.lax.broadcasted_iota(jnp.int32, (rows, LANES), 1)
        m1 = (lane & 1) != 0
        m2 = (lane & 2) != 0
        start = tok0 + PAD
        q = [q_v[j, pl.ds(start, rows), :] for j in range(NT)]
        ls = []
        for w in range(W):
            acc = None
            for j in range(NT):
                p = q[j] * k_v[j, pl.ds(start - DIL * w, rows), :]
                acc = p if acc is None else acc + p
            acc = acc + jnp.where(m1, pltpu.roll(acc, 1, 1), pltpu.roll(acc, LANES - 1, 1))
            acc = acc + jnp.where(m2, pltpu.roll(acc, 2, 1), pltpu.roll(acc, LANES - 2, 1))
            if masked and w > 0:
                tok = jax.lax.broadcasted_iota(jnp.int32, (rows, LANES), 0) + tok0
                acc = jnp.where(tok >= DIL * w, acc, MASK_VALUE)
            ls.append(acc)
        mx = functools.reduce(jnp.maximum, ls)
        es = [jnp.exp(l - mx) for l in ls]
        inv = 1.0 / functools.reduce(lambda a, b: a + b, es)
        ps = [e * inv for e in es]
        o = []
        for j in range(NT):
            acc = None
            for w in range(W):
                p = ps[w] * v_v[j, pl.ds(start - DIL * w, rows), :]
                acc = p if acc is None else acc + p
            o.append(acc)
        o = _swap_tile_lane_bits(o)
        store(jnp.concatenate(o, axis=1).astype(bf16))

    x_copy(0).start()
    wk_copy(0).start()

    zeros = jnp.zeros((NT, PAD, LANES), f32)
    k_v[:, 0:PAD, :] = zeros
    v_v[:, 0:PAD, :] = zeros

    x_copy(0).wait()
    wk_copy(1).start()
    wk_copy(2).start()
    do_ln(0, 0, TA)
    wk_copy(0).wait()
    wk_copy(3).start()
    permute_weight(wk_v, 0, KS)

    def k0_step(s, first):
        ks = pl.ds(blk(s, KS), KS)
        part = jnp.dot(xn_v[0:TA, ks], wk_v[ks, :], preferred_element_type=f32)
        for j in range(NT):
            p = part[:, j * LANES:(j + 1) * LANES]
            dst = k_v.at[j, PAD:PAD + TA, :]
            if first is None:
                dst[...] = dst[...] + p
            else:
                dst[...] = jnp.where(first, p, dst[...] + p)

    def body_p(s, carry):
        wk_copy(s + 1).wait()
        x_copy(s + 1).start()
        wv_copy(s).start()
        k0_step(s, s == 0)
        permute_weight(wk_v, s + 1, KS)
        return carry

    jax.lax.fori_loop(0, NK - 1, body_p, 0)
    x_copy(1).wait()
    wv_copy(0).wait()
    wq_copy(0).start()
    k0_step(NK - 1, None)
    permute_weight(wv_v, 0, WS)
    do_ln(TA, 0, TA)

    def body_k(i, carry):
        x_copy(i + 1).wait()
        wv_copy(i).wait()

        @pl.when(i + 2 < NB)
        def _():
            x_copy(i + 3).start()
            wv_copy(i + 2).start()

        wq_copy(i).start()
        start = blk(i, TA)
        project(wk_v, k_v, start)
        do_ln(start + TA, 0, TA)
        permute_weight(wv_v, i, WS)
        return carry

    jax.lax.fori_loop(1, NB, body_k, 0)
    for cp in w_copies:
        cp.start()

    def body_v(i, carry):
        wq_copy(i).wait()
        project(wv_v, v_v, blk(i, TA))
        permute_weight(wq_v, i, WS)
        return carry

    jax.lax.fori_loop(0, NB, body_v, 0)

    def body_q(i, carry):
        tok0 = pl.multiple_of(jnp.clip((i - 1) * RP, 0, TB - RP), 8)

        def store(o):
            o_v[pl.ds(tok0, RP), :] = o

        attention(tok0, RP, True, store)
        project(wq_v, q_v, blk(i, TA), DH ** -0.5)
        return carry

    jax.lax.fori_loop(0, NB, body_q, 0)

    for cp in w_copies:
        cp.wait()

    def body_b(i, carry):
        base = blk(i, TB)
        rows = pl.ds(base, TB)
        nbase = pl.multiple_of(jnp.minimum(i + 1, NB - 1) * TB, TB)
        oc_v[...] = o_v[...]
        nc = F // FC
        pieces = list(range(0, TB, RA))
        acc = None
        for c in range(nc):
            sl = slice(c * FC, (c + 1) * FC)
            g = jnp.dot(xn_v[rows, :], w1_v[:, sl], preferred_element_type=f32)
            u = jnp.dot(xn_v[rows, :], w3_v[:, sl], preferred_element_type=f32)
            h = (_silu(g) * u).astype(bf16)
            d = jnp.dot(h, w2_v[sl, :], preferred_element_type=f32)
            acc = d if acc is None else acc + d
            lo = (len(pieces) * c) // nc
            hi = (len(pieces) * (c + 1)) // nc
            for r in pieces[lo:hi]:
                def store(o, r=r):
                    o_v[pl.ds(r, RA), :] = o
                attention(nbase + r, RA, False, store)
        gate = _silu(acc)
        s = jnp.dot(oc_v[...], wo_v[...], preferred_element_type=f32)
        out_v[rows, :] = (x_v[rows, :].astype(f32) + s * gate).astype(bf16)
        out_copy(i).start()
        return carry

    jax.lax.fori_loop(0, NB, body_b, 0)
    for i in range(NB):
        out_copy(i).wait()


@jax.jit
def pallas_recurrent_scan__sliding_local_dilated__glu_gated_swiglu__prompt_kernel(
    A_x: jax.Array,
    A_wqkv: jax.Array,
    A_wo: jax.Array,
    B_x: jax.Array,
    B_w1: jax.Array,
    B_w3: jax.Array,
    B_w2: jax.Array,
):
    x = A_x.reshape(S, D)
    any_spec = pl.BlockSpec(memory_space=pl.ANY)
    out = pl.pallas_call(
        _kernel,
        out_shape=jax.ShapeDtypeStruct((S, D), bf16),
        in_specs=[any_spec] * 6,
        out_specs=any_spec,
        scratch_shapes=[
            pltpu.VMEM((S + TA, D), bf16),
            pltpu.VMEM((S + TA, D), bf16),
            pltpu.VMEM((D, D), bf16),
            pltpu.VMEM((D, D), bf16),
            pltpu.VMEM((D, D), bf16),
            pltpu.VMEM((D, D), bf16),
            pltpu.VMEM((D, F), bf16),
            pltpu.VMEM((D, F), bf16),
            pltpu.VMEM((F, D), bf16),
            pltpu.VMEM((NT, PAD + S, LANES), f32),
            pltpu.VMEM((NT, PAD + S, LANES), f32),
            pltpu.VMEM((NT, PAD + S, LANES), f32),
            pltpu.VMEM((TB, D), bf16),
            pltpu.VMEM((TB, D), bf16),
            pltpu.VMEM((S, D), bf16),
            pltpu.SemaphoreType.DMA((NB + 1,)),
            pltpu.SemaphoreType.DMA((NB,)),
            pltpu.SemaphoreType.DMA((NK,)),
            pltpu.SemaphoreType.DMA((NB,)),
            pltpu.SemaphoreType.DMA((4,)),
            pltpu.SemaphoreType.DMA((NB,)),
        ],
        compiler_params=pltpu.CompilerParams(vmem_limit_bytes=120 * 1024 * 1024),
    )(x, A_wqkv, A_wo, B_w1, B_w3, B_w2)
    return out.reshape(1, S, D)
```

```python
import functools

import jax
import jax.numpy as jnp
from jax.experimental import pallas as pl
from jax.experimental.pallas import tpu as pltpu

S = 2048
D = 1024
F = 3584
H = 32
DH = D // H
W = 8
DIL = 2
PAD = 16
LANES = 128
NT = D // LANES
TB = 256
NB = S // TB
FC = 512
KU = 256
NU = 3 * D // KU
PR = 128
RA = 16
RP = 40
EPS = 1e-5
MASK_VALUE = -1e9
Q_SCALE = DH ** -0.5

f32 = jnp.float32
bf16 = jnp.bfloat16
u32 = jnp.uint32


def _swap_tile_lane_bits(tiles):
    lane = jax.lax.broadcasted_iota(jnp.int32, tiles[0].shape, 1)
    r = [tiles[0]] + [pltpu.roll(tiles[t], 4 * t, 1) for t in range(1, NT)]
    u = [r[(-k) % NT] for k in range(NT)]
    for b in range(3):
        m = (lane & (4 << b)) != 0
        u = [jnp.where(m, u[(k - (1 << b)) % NT], u[k]) for k in range(NT)]
    return [u[0]] + [pltpu.roll(u[t], LANES - 4 * t, 1) for t in range(1, NT)]


def _layernorm(x):
    x = x.astype(f32)
    m = jnp.mean(x, axis=-1, keepdims=True)
    xc = x - m
    v = jnp.mean(xc * xc, axis=-1, keepdims=True)
    return (xc * jax.lax.rsqrt(v + EPS)).astype(bf16)


def _silu(x):
    h = 0.5 * x
    return h + h * jnp.tanh(h)


def _kernel(x_hbm, wqkv_hbm, wo_hbm, w1_hbm, w3_hbm, w2_hbm, out_hbm,
            x_v, xn_v, wa_v, wp_v, wo_v, w1_v, w3_v, w2_v,
            kvq0_v, q_v, k_v, v_v, o_v, oc_v, out_v,
            in_sem, out_sem):

    X_SEM, WA_SEM, W_SEM = 0, NB + 1, NB + 1 + NU

    def blk(i, n):
        return i * n if isinstance(i, int) else pl.multiple_of(i * n, n)

    def x_copy(b):
        src = min(b, NB - 1) if isinstance(b, int) else jnp.minimum(b, NB - 1)
        return pltpu.make_async_copy(
            x_hbm.at[pl.ds(blk(src, TB), TB)], x_v.at[pl.ds(blk(b, TB), TB)], in_sem.at[X_SEM + b])

    def wa_copy(n):
        per = D // KU
        col = ((n // per + 1) % 3)
        return pltpu.make_async_copy(
            wqkv_hbm.at[pl.ds(blk(n % per, KU), KU), pl.ds(blk(col, D), D)],
            wa_v.at[pl.ds(blk(n, KU), KU)], in_sem.at[WA_SEM + n])

    w_copies = [
        pltpu.make_async_copy(w1_hbm, w1_v, in_sem.at[W_SEM + 0]),
        pltpu.make_async_copy(w3_hbm, w3_v, in_sem.at[W_SEM + 1]),
        pltpu.make_async_copy(w2_hbm, w2_v, in_sem.at[W_SEM + 2]),
        pltpu.make_async_copy(wo_hbm, wo_v, in_sem.at[W_SEM + 3]),
    ]

    def out_copy(i):
        rows = pl.ds(blk(i, TB), TB)
        return pltpu.make_async_copy(out_v.at[rows], out_hbm.at[rows], out_sem.at[i])

    def permute_weight(n, units):
        for r in range(0, units * KU, PR):
            rows = pl.ds(blk(n, KU) + r, PR)
            prows = pl.ds(blk(n, KU // 2) + r // 2, PR // 2)
            tiles = [pltpu.bitcast(wa_v[rows, j * LANES:(j + 1) * LANES], u32)
                     for j in range(NT)]
            tiles = _swap_tile_lane_bits(tiles)
            for j in range(NT):
                wp_v[prows, j * LANES:(j + 1) * LANES] = tiles[j]

    def half(start):
        return start // 2 if isinstance(start, int) else pl.multiple_of(start // 2, TB // 2)

    def do_ln(start):
        for r in range(0, TB, 32):
            xn = _layernorm(x_v[pl.ds(start + r, 32), :])
            xn_v[pl.ds(half(start) + r // 2, 16), :] = pltpu.bitcast(xn, u32)

    def xn_block(start):
        return pltpu.bitcast(xn_v[pl.ds(half(start), TB // 2), :], bf16)

    def project(sec, dst, start, scale=None):
        w = pltpu.bitcast(wp_v[sec * D // 2:(sec + 1) * D // 2, :], bf16)
        res = jnp.dot(xn_block(start), w, preferred_element_type=f32)
        if scale is not None:
            res = res * scale
        for j in range(NT):
            dst[j, pl.ds(PAD + start, TB), :] = res[:, j * LANES:(j + 1) * LANES]

    def attention(q_ref, k_ref, v_ref, tok0, rows, first_block, store):
        lane = jax.lax.broadcasted_iota(jnp.int32, (rows, LANES), 1)
        m1 = (lane & 1) != 0
        m2 = (lane & 2) != 0
        start = tok0 + PAD
        q = [q_ref[j, pl.ds(start, rows), :] for j in range(NT)]
        if first_block:
            q = [t * Q_SCALE for t in q]
        ls = []
        for w in range(W):
            acc = None
            for j in range(NT):
                p = q[j] * k_ref[j, pl.ds(start - DIL * w, rows), :]
                acc = p if acc is None else acc + p
            acc = acc + jnp.where(m1, pltpu.roll(acc, 1, 1), pltpu.roll(acc, LANES - 1, 1))
            acc = acc + jnp.where(m2, pltpu.roll(acc, 2, 1), pltpu.roll(acc, LANES - 2, 1))
            if first_block and w > 0:
                tok = jax.lax.broadcasted_iota(jnp.int32, (rows, LANES), 0) + tok0
                acc = jnp.where(tok >= DIL * w, acc, MASK_VALUE)
            ls.append(acc)
        mx = functools.reduce(jnp.maximum, ls)
        es = [jnp.exp(l - mx) for l in ls]
        inv = 1.0 / functools.reduce(lambda a, b: a + b, es)
        ps = [e * inv for e in es]
        o = []
        for j in range(NT):
            acc = None
            for w in range(W):
                p = ps[w] * v_ref[j, pl.ds(start - DIL * w, rows), :]
                acc = p if acc is None else acc + p
            o.append(acc)
        o = _swap_tile_lane_bits(o)
        store(jnp.concatenate(o, axis=1).astype(bf16))

    x_copy(0).start()
    for n in range(NU):
        wa_copy(n).start()
    for b in range(1, NB + 1):
        x_copy(b).start()
    for cp in w_copies:
        cp.start()

    kvq0_v[0:2, :, 0:PAD, :] = jnp.zeros((2, NT, PAD, LANES), f32)

    x_copy(0).wait()
    do_ln(0)
    wa_copy(0).wait()
    permute_weight(0, 1)

    def k0_step(n, units):
        per = D // KU
        ks = pl.ds(blk(n % per, KU), units * KU)
        part = jnp.dot(pltpu.bitcast(xn_v[0:TB // 2, ks], bf16),
                       pltpu.bitcast(wp_v[pl.ds(blk(n, KU // 2), units * KU // 2), :], bf16),
                       preferred_element_type=f32)
        for j in range(NT):
            p = part[:, j * LANES:(j + 1) * LANES]
            dst = kvq0_v.at[n // per, j, PAD:PAD + TB, :]
            if isinstance(n, int):
                dst[...] = p if n % per == 0 else dst[...] + p
            else:
                dst[...] = jnp.where(n % per == 0, p, dst[...] + p)

    def body_p1(n, carry):
        wa_copy(n + 1).wait()
        k0_step(n, 1)
        permute_weight(n + 1, 1)
        return carry

    jax.lax.fori_loop(0, 3, body_p1, 0)
    wa_copy(4).wait()
    wa_copy(5).wait()
    k0_step(3, 1)
    permute_weight(4, 2)

    def body_p2(m, carry):
        n = 4 + 2 * m
        wa_copy(n + 2).wait()
        wa_copy(n + 3).wait()

        k0_step(n, 2)
        permute_weight(n + 2, 2)
        return carry

    jax.lax.fori_loop(0, 3, body_p2, 0)
    x_copy(1).wait()
    k0_step(NU - 2, 2)
    do_ln(TB)
    k_v[:, TB:TB + PAD, :] = kvq0_v[0, :, TB:TB + PAD, :]
    v_v[:, TB:TB + PAD, :] = kvq0_v[1, :, TB:TB + PAD, :]

    def body_a(i, carry):
        x_copy(i + 1).wait()

        start = blk(i, TB)
        project(0, k_v, start)
        project(1, v_v, start)
        project(2, q_v, start, Q_SCALE)
        do_ln(start + TB)
        tok0 = pl.multiple_of(jnp.minimum((i - 1) * RP, TB - RP), 8)

        def store(o):
            o_v[pl.ds(tok0, RP), :] = o

        attention(kvq0_v.at[2], kvq0_v.at[0], kvq0_v.at[1], tok0, RP, True, store)
        return carry

    jax.lax.fori_loop(1, NB, body_a, 0)

    for cp in w_copies:
        cp.wait()

    def body_b(i, carry):
        base = blk(i, TB)
        rows = pl.ds(base, TB)
        nbase = pl.multiple_of(jnp.minimum(i + 1, NB - 1) * TB, TB)
        oc_v[...] = o_v[...]
        nc = F // FC
        pieces = list(range(0, TB, RA))
        acc = None
        for c in range(nc):
            sl = slice(c * FC, (c + 1) * FC)
            g = jnp.dot(xn_block(base), w1_v[:, sl], preferred_element_type=f32)
            u = jnp.dot(xn_block(base), w3_v[:, sl], preferred_element_type=f32)
            h = (_silu(g) * u).astype(bf16)
            d = jnp.dot(h, w2_v[sl, :], preferred_element_type=f32)
            acc = d if acc is None else acc + d
            lo = (len(pieces) * c) // nc
            hi = (len(pieces) * (c + 1)) // nc
            for r in pieces[lo:hi]:
                def store(o, r=r):
                    o_v[pl.ds(r, RA), :] = o
                attention(q_v, k_v, v_v, nbase + r, RA, False, store)
        gate = _silu(acc)
        s = jnp.dot(oc_v[...], wo_v[...], preferred_element_type=f32)
        out_v[rows, :] = (x_v[rows, :].astype(f32) + s * gate).astype(bf16)
        out_copy(i).start()
        return carry

    jax.lax.fori_loop(0, NB, body_b, 0)
    for i in range(NB):
        out_copy(i).wait()


@jax.jit
def pallas_recurrent_scan__sliding_local_dilated__glu_gated_swiglu__prompt_kernel(
    A_x: jax.Array,
    A_wqkv: jax.Array,
    A_wo: jax.Array,
    B_x: jax.Array,
    B_w1: jax.Array,
    B_w3: jax.Array,
    B_w2: jax.Array,
):
    x = A_x.reshape(S, D)
    any_spec = pl.BlockSpec(memory_space=pl.ANY)
    out = pl.pallas_call(
        _kernel,
        out_shape=jax.ShapeDtypeStruct((S, D), bf16),
        in_specs=[any_spec] * 6,
        out_specs=any_spec,
        scratch_shapes=[
            pltpu.VMEM((S + TB, D), bf16),
            pltpu.VMEM(((S + TB) // 2, D), u32),
            pltpu.VMEM((3 * D, D), bf16),
            pltpu.VMEM((3 * D // 2, D), u32),
            pltpu.VMEM((D, D), bf16),
            pltpu.VMEM((D, F), bf16),
            pltpu.VMEM((D, F), bf16),
            pltpu.VMEM((F, D), bf16),
            pltpu.VMEM((3, NT, PAD + TB, LANES), f32),
            pltpu.VMEM((NT, PAD + S, LANES), f32),
            pltpu.VMEM((NT, PAD + S, LANES), f32),
            pltpu.VMEM((NT, PAD + S, LANES), f32),
            pltpu.VMEM((TB, D), bf16),
            pltpu.VMEM((TB, D), bf16),
            pltpu.VMEM((S, D), bf16),
            pltpu.SemaphoreType.DMA((NB + 1 + NU + 4,)),
            pltpu.SemaphoreType.DMA((NB,)),
        ],
        compiler_params=pltpu.CompilerParams(vmem_limit_bytes=120 * 1024 * 1024),
    )(x, A_wqkv, A_wo, B_w1, B_w3, B_w2)
    return out.reshape(1, S, D)
```

```python
import functools

import jax
import jax.numpy as jnp
from jax.experimental import pallas as pl
from jax.experimental.pallas import tpu as pltpu

S = 2048
D = 1024
F = 3584
H = 32
DH = D // H
W = 8
DIL = 2
PAD = 16
LANES = 128
NT = D // LANES
TB = 256
NB = S // TB
FC = 512
KU = 256
NU = 3 * D // KU
PR = 128
RA = 8
LNR = 32
EPS = 1e-5
MASK_VALUE = -1e9
Q_SCALE = DH ** -0.5 * 1.4426950408889634

f32 = jnp.float32
bf16 = jnp.bfloat16
u32 = jnp.uint32


def _swap_tile_lane_bits(tiles):
    lane = jax.lax.broadcasted_iota(jnp.int32, tiles[0].shape, 1)
    r = [tiles[0]] + [pltpu.roll(tiles[t], 4 * t, 1) for t in range(1, NT)]
    u = [r[(-k) % NT] for k in range(NT)]
    for b in range(3):
        m = (lane & (4 << b)) != 0
        u = [jnp.where(m, u[(k - (1 << b)) % NT], u[k]) for k in range(NT)]
    return [u[0]] + [pltpu.roll(u[t], LANES - 4 * t, 1) for t in range(1, NT)]


def _layernorm(x):
    x = x.astype(f32)
    m = jnp.mean(x, axis=-1, keepdims=True)
    xc = x - m
    v = jnp.mean(xc * xc, axis=-1, keepdims=True)
    return (xc * jax.lax.rsqrt(v + EPS)).astype(bf16)


def _silu(x):
    h = 0.5 * x
    return h + h * jnp.tanh(h)


def _kernel(x_hbm, wqkv_hbm, wo_hbm, w1_hbm, w3_hbm, w2_hbm, out_hbm,
            x_v, xn_v, wa_v, wp_v, wo_v, w1_v, w3_v, w2_v,
            kvq0_v, q_v, k_v, v_v, o_v, oc_v, out_v,
            in_sem, out_sem):

    X_SEM, WA_SEM, W_SEM = 0, NB + 1, NB + 1 + NU

    def blk(i, n):
        return i * n if isinstance(i, int) else pl.multiple_of(i * n, n)

    def x_copy(b):
        src = min(b, NB - 1) if isinstance(b, int) else jnp.minimum(b, NB - 1)
        return pltpu.make_async_copy(
            x_hbm.at[pl.ds(blk(src, TB), TB)], x_v.at[pl.ds(blk(b, TB), TB)], in_sem.at[X_SEM + b])

    def wa_copy(n):
        per = D // KU
        col = ((n // per + 1) % 3)
        return pltpu.make_async_copy(
            wqkv_hbm.at[pl.ds(blk(n % per, KU), KU), pl.ds(blk(col, D), D)],
            wa_v.at[pl.ds(blk(n, KU), KU)], in_sem.at[WA_SEM + n])

    w_copies = [
        pltpu.make_async_copy(w1_hbm, w1_v, in_sem.at[W_SEM + 0]),
        pltpu.make_async_copy(w3_hbm, w3_v, in_sem.at[W_SEM + 1]),
        pltpu.make_async_copy(w2_hbm, w2_v, in_sem.at[W_SEM + 2]),
        pltpu.make_async_copy(wo_hbm, wo_v, in_sem.at[W_SEM + 3]),
    ]

    def out_copy(i):
        rows = pl.ds(blk(i, TB), TB)
        return pltpu.make_async_copy(out_v.at[rows], out_hbm.at[rows], out_sem.at[i])

    def permute_weight(n, units):
        for r in range(0, units * KU, PR):
            rows = pl.ds(blk(n, KU) + r, PR)
            prows = pl.ds(blk(n, KU // 2) + r // 2, PR // 2)
            tiles = [pltpu.bitcast(wa_v[rows, j * LANES:(j + 1) * LANES], u32)
                     for j in range(NT)]
            tiles = _swap_tile_lane_bits(tiles)
            for j in range(NT):
                wp_v[prows, j * LANES:(j + 1) * LANES] = tiles[j]

    def half(start):
        return start // 2 if isinstance(start, int) else pl.multiple_of(start // 2, TB // 2)

    def do_ln(start):
        for r in range(0, TB, LNR):
            xn = _layernorm(x_v[pl.ds(start + r, LNR), :])
            xn_v[pl.ds(half(start) + r // 2, LNR // 2), :] = pltpu.bitcast(xn, u32)

    def xn_block(start):
        return pltpu.bitcast(xn_v[pl.ds(half(start), TB // 2), :], bf16)

    def project(sec, dst, start, scale=None):
        w = pltpu.bitcast(wp_v[sec * D // 2:(sec + 1) * D // 2, :], bf16)
        res = jnp.dot(xn_block(start), w, preferred_element_type=f32)
        if scale is not None:
            res = res * scale
        for j in range(NT):
            dst[j, pl.ds(PAD + start, TB), :] = res[:, j * LANES:(j + 1) * LANES]

    def attention(q_ref, k_ref, v_ref, tok0, rows, first_block, store):
        lane = jax.lax.broadcasted_iota(jnp.int32, (rows, LANES), 1)
        m1 = (lane & 1) != 0
        m2 = (lane & 2) != 0
        start = tok0 + PAD
        q = [q_ref[j, pl.ds(start, rows), :] for j in range(NT)]
        if first_block:
            q = [t * Q_SCALE for t in q]
        ls = []
        for w in range(W):
            acc = None
            for j in range(NT):
                p = q[j] * k_ref[j, pl.ds(start - DIL * w, rows), :]
                acc = p if acc is None else acc + p
            acc = acc + jnp.where(m1, pltpu.roll(acc, 1, 1), pltpu.roll(acc, LANES - 1, 1))
            acc = acc + jnp.where(m2, pltpu.roll(acc, 2, 1), pltpu.roll(acc, LANES - 2, 1))
            if first_block and w > 0:
                tok = jax.lax.broadcasted_iota(jnp.int32, (rows, LANES), 0) + tok0
                acc = jnp.where(tok >= DIL * w, acc, MASK_VALUE)
            ls.append(acc)
        mx = functools.reduce(jnp.maximum, ls)
        es = [jnp.exp2(l - mx) for l in ls]
        inv = 1.0 / functools.reduce(lambda a, b: a + b, es)
        ps = [e * inv for e in es]
        o = []
        for j in range(NT):
            acc = None
            for w in range(W):
                p = ps[w] * v_ref[j, pl.ds(start - DIL * w, rows), :]
                acc = p if acc is None else acc + p
            o.append(acc)
        o = _swap_tile_lane_bits(o)
        store(jnp.concatenate(o, axis=1).astype(bf16))

    x_copy(0).start()
    for n in range(NU):
        wa_copy(n).start()
    for b in range(1, NB + 1):
        x_copy(b).start()
    for cp in w_copies:
        cp.start()

    kvq0_v[0:2, :, 0:PAD, :] = jnp.zeros((2, NT, PAD, LANES), f32)

    x_copy(0).wait()
    do_ln(0)
    wa_copy(0).wait()
    permute_weight(0, 1)

    def k0_step(n, units):
        per = D // KU
        ks = pl.ds(blk(n % per, KU), units * KU)
        part = jnp.dot(pltpu.bitcast(xn_v[0:TB // 2, ks], bf16),
                       pltpu.bitcast(wp_v[pl.ds(blk(n, KU // 2), units * KU // 2), :], bf16),
                       preferred_element_type=f32)
        for j in range(NT):
            p = part[:, j * LANES:(j + 1) * LANES]
            dst = kvq0_v.at[n // per, j, PAD:PAD + TB, :]
            if isinstance(n, int):
                dst[...] = p if n % per == 0 else dst[...] + p
            else:
                dst[...] = jnp.where(n % per == 0, p, dst[...] + p)

    def body_p(n, carry):
        wa_copy(n + 1).wait()
        k0_step(n, 1)
        permute_weight(n + 1, 1)
        return carry

    jax.lax.fori_loop(0, NU - 1, body_p, 0)
    x_copy(1).wait()
    k0_step(NU - 1, 1)
    do_ln(TB)
    k_v[:, TB:TB + PAD, :] = kvq0_v[0, :, TB:TB + PAD, :]
    v_v[:, TB:TB + PAD, :] = kvq0_v[1, :, TB:TB + PAD, :]

    def body_a(i, carry):
        x_copy(i + 1).wait()

        start = blk(i, TB)

        def att0():
            base0 = pl.multiple_of((i - 1) * 32, 32)
            plist = [(base0 + r, RA) for r in range(0, 32, RA)]
            plist.append((pl.multiple_of(jnp.minimum(TB - 32 + (i - 1) * 8, TB - 8), 8), 8))
            for tok0, rows in plist:

                def store(o, tok0=tok0, rows=rows):
                    o_v[pl.ds(pl.multiple_of(tok0, 8), rows), :] = o

                attention(kvq0_v.at[2], kvq0_v.at[0], kvq0_v.at[1], tok0, rows, True, store)

        project(0, k_v, start)
        project(1, v_v, start)
        project(2, q_v, start, Q_SCALE)
        att0()
        do_ln(start + TB)
        return carry

    jax.lax.fori_loop(1, NB, body_a, 0)

    for cp in w_copies:
        cp.wait()

    def body_b(i, carry):
        base = blk(i, TB)
        rows = pl.ds(base, TB)
        nbase = pl.multiple_of(jnp.minimum(i + 1, NB - 1) * TB, TB)
        oc_v[...] = o_v[...]
        nc = F // FC
        pieces = list(range(0, TB, RA))

        def att(rs):
            for r in rs:
                def store(o, r=r):
                    o_v[pl.ds(r, RA), :] = o
                attention(q_v, k_v, v_v, nbase + r, RA, False, store)

        acc = None
        for c in range(nc):
            sl = slice(c * FC, (c + 1) * FC)
            g = jnp.dot(xn_block(base), w1_v[:, sl], preferred_element_type=f32)
            u = jnp.dot(xn_block(base), w3_v[:, sl], preferred_element_type=f32)
            h = (_silu(g) * u).astype(bf16)
            d = jnp.dot(h, w2_v[sl, :], preferred_element_type=f32)
            acc = d if acc is None else acc + d
            att(pieces[(len(pieces) * c) // nc:(len(pieces) * (c + 1)) // nc])
        gate = _silu(acc)
        s = jnp.dot(oc_v[...], wo_v[...], preferred_element_type=f32)
        out_v[rows, :] = (x_v[rows, :].astype(f32) + s * gate).astype(bf16)
        out_copy(i).start()
        return carry

    jax.lax.fori_loop(0, NB, body_b, 0)
    for i in range(NB):
        out_copy(i).wait()


@jax.jit
def pallas_recurrent_scan__sliding_local_dilated__glu_gated_swiglu__prompt_kernel(
    A_x: jax.Array,
    A_wqkv: jax.Array,
    A_wo: jax.Array,
    B_x: jax.Array,
    B_w1: jax.Array,
    B_w3: jax.Array,
    B_w2: jax.Array,
):
    x = A_x.reshape(S, D)
    any_spec = pl.BlockSpec(memory_space=pl.ANY)
    out = pl.pallas_call(
        _kernel,
        out_shape=jax.ShapeDtypeStruct((S, D), bf16),
        in_specs=[any_spec] * 6,
        out_specs=any_spec,
        scratch_shapes=[
            pltpu.VMEM((S + TB, D), bf16),
            pltpu.VMEM(((S + TB) // 2, D), u32),
            pltpu.VMEM((3 * D, D), bf16),
            pltpu.VMEM((3 * D // 2, D), u32),
            pltpu.VMEM((D, D), bf16),
            pltpu.VMEM((D, F), bf16),
            pltpu.VMEM((D, F), bf16),
            pltpu.VMEM((F, D), bf16),
            pltpu.VMEM((3, NT, PAD + TB, LANES), f32),
            pltpu.VMEM((NT, PAD + S, LANES), f32),
            pltpu.VMEM((NT, PAD + S, LANES), f32),
            pltpu.VMEM((NT, PAD + S, LANES), f32),
            pltpu.VMEM((TB, D), bf16),
            pltpu.VMEM((TB, D), bf16),
            pltpu.VMEM((S, D), bf16),
            pltpu.SemaphoreType.DMA((NB + 1 + NU + 4,)),
            pltpu.SemaphoreType.DMA((NB,)),
        ],
        compiler_params=pltpu.CompilerParams(vmem_limit_bytes=120 * 1024 * 1024),
    )(x, A_wqkv, A_wo, B_w1, B_w3, B_w2)
    return out.reshape(1, S, D)
```

```python
import functools

import jax
import jax.numpy as jnp
from jax.experimental import pallas as pl
from jax.experimental.pallas import tpu as pltpu

S = 2048
D = 1024
F = 3584
H = 32
DH = D // H
W = 8
DIL = 2
PAD = 16
LANES = 128
NT = D // LANES
TB = 256
NB = S // TB
FC = 512
KU = 256
NU = 3 * D // KU
PR = 128
RA = 8
LNR = 32
EPS = 1e-5
MASK_VALUE = -1e9
Q_SCALE = DH ** -0.5 * 1.4426950408889634

f32 = jnp.float32
bf16 = jnp.bfloat16
u32 = jnp.uint32


def _swap_tile_lane_bits(tiles):
    lane = jax.lax.broadcasted_iota(jnp.int32, tiles[0].shape, 1)
    r = [tiles[0]] + [pltpu.roll(tiles[t], 4 * t, 1) for t in range(1, NT)]
    u = [r[(-k) % NT] for k in range(NT)]
    for b in range(3):
        m = (lane & (4 << b)) != 0
        u = [jnp.where(m, u[(k - (1 << b)) % NT], u[k]) for k in range(NT)]
    return [u[0]] + [pltpu.roll(u[t], LANES - 4 * t, 1) for t in range(1, NT)]


def _layernorm(x):
    x = x.astype(f32)
    m = jnp.mean(x, axis=-1, keepdims=True)
    xc = x - m
    v = jnp.mean(xc * xc, axis=-1, keepdims=True)
    return (xc * jax.lax.rsqrt(v + EPS)).astype(bf16)


def _silu(x):
    h = 0.5 * x
    return h + h * jnp.tanh(h)


def _kernel(x_hbm, wqkv_hbm, wo_hbm, w1_hbm, w3_hbm, w2_hbm, out_hbm,
            x_v, xn_v, wa_v, wp_v, wo_v, w1_v, w3_v, w2_v,
            kvq0_v, q_v, k_v, v_v, o_v, oc_v, out_v,
            in_sem, out_sem):

    X_SEM, WA_SEM, W_SEM = 0, NB + 1, NB + 1 + NU

    def blk(i, n):
        return i * n if isinstance(i, int) else pl.multiple_of(i * n, n)

    def x_copy(b):
        src = min(b, NB - 1) if isinstance(b, int) else jnp.minimum(b, NB - 1)
        return pltpu.make_async_copy(
            x_hbm.at[pl.ds(blk(src, TB), TB)], x_v.at[pl.ds(blk(b, TB), TB)], in_sem.at[X_SEM + b])

    def wa_copy(n):
        per = D // KU
        col = ((n // per + 1) % 3)
        return pltpu.make_async_copy(
            wqkv_hbm.at[pl.ds(blk(n % per, KU), KU), pl.ds(blk(col, D), D)],
            wa_v.at[pl.ds(blk(n, KU), KU)], in_sem.at[WA_SEM + n])

    w_copies = [
        pltpu.make_async_copy(w1_hbm, w1_v, in_sem.at[W_SEM + 0]),
        pltpu.make_async_copy(w3_hbm, w3_v, in_sem.at[W_SEM + 1]),
        pltpu.make_async_copy(w2_hbm, w2_v, in_sem.at[W_SEM + 2]),
        pltpu.make_async_copy(wo_hbm, wo_v, in_sem.at[W_SEM + 3]),
    ]

    def out_copy(i):
        rows = pl.ds(blk(i, TB), TB)
        return pltpu.make_async_copy(out_v.at[rows], out_hbm.at[rows], out_sem.at[i])

    def permute_weight(n, units):
        for r in range(0, units * KU, PR):
            rows = pl.ds(blk(n, KU) + r, PR)
            prows = pl.ds(blk(n, KU // 2) + r // 2, PR // 2)
            tiles = [pltpu.bitcast(wa_v[rows, j * LANES:(j + 1) * LANES], u32)
                     for j in range(NT)]
            tiles = _swap_tile_lane_bits(tiles)
            for j in range(NT):
                wp_v[prows, j * LANES:(j + 1) * LANES] = tiles[j]

    def half(start):
        return start // 2 if isinstance(start, int) else pl.multiple_of(start // 2, TB // 2)

    def do_ln(start):
        for r in range(0, TB, LNR):
            xn = _layernorm(x_v[pl.ds(start + r, LNR), :])
            xn_v[pl.ds(half(start) + r // 2, LNR // 2), :] = pltpu.bitcast(xn, u32)

    def xn_block(start):
        return pltpu.bitcast(xn_v[pl.ds(half(start), TB // 2), :], bf16)

    def project(sec, dst, start, scale=None):
        w = pltpu.bitcast(wp_v[sec * D // 2:(sec + 1) * D // 2, :], bf16)
        res = jnp.dot(xn_block(start), w, preferred_element_type=f32)
        if scale is not None:
            res = res * scale
        for j in range(NT):
            dst[j, pl.ds(PAD + start, TB), :] = res[:, j * LANES:(j + 1) * LANES]

    def attention(q_ref, k_ref, v_ref, tok0, rows, first_block, store):
        lane = jax.lax.broadcasted_iota(jnp.int32, (rows, LANES), 1)
        m1 = (lane & 1) != 0
        m2 = (lane & 2) != 0
        start = tok0 + PAD
        q = [q_ref[j, pl.ds(start, rows), :] for j in range(NT)]
        if first_block:
            q = [t * Q_SCALE for t in q]
        ls = []
        for w in range(W):
            acc = None
            for j in range(NT):
                p = q[j] * k_ref[j, pl.ds(start - DIL * w, rows), :]
                acc = p if acc is None else acc + p
            acc = acc + jnp.where(m1, pltpu.roll(acc, 1, 1), pltpu.roll(acc, LANES - 1, 1))
            acc = acc + jnp.where(m2, pltpu.roll(acc, 2, 1), pltpu.roll(acc, LANES - 2, 1))
            if first_block and w > 0:
                tok = jax.lax.broadcasted_iota(jnp.int32, (rows, LANES), 0) + tok0
                acc = jnp.where(tok >= DIL * w, acc, MASK_VALUE)
            ls.append(acc)
        mx = functools.reduce(jnp.maximum, ls)
        es = [jnp.exp2(l - mx) for l in ls]
        inv = 1.0 / functools.reduce(lambda a, b: a + b, es)
        ps = [e * inv for e in es]
        o = []
        for j in range(NT):
            acc = None
            for w in range(W):
                p = ps[w] * v_ref[j, pl.ds(start - DIL * w, rows), :]
                acc = p if acc is None else acc + p
            o.append(acc)
        o = _swap_tile_lane_bits(o)
        store(jnp.concatenate(o, axis=1).astype(bf16))

    x_copy(0).start()
    for n in range(NU):
        wa_copy(n).start()
    for b in range(1, NB + 1):
        x_copy(b).start()
    for cp in w_copies:
        cp.start()

    def zero_body(z, carry):
        kvq0_v[z] = jnp.zeros((NT, PAD + TB, LANES), f32)
        return carry

    jax.lax.fori_loop(0, 3, zero_body, 0)

    x_copy(0).wait()
    do_ln(0)
    wa_copy(0).wait()
    permute_weight(0, 1)

    def k0_step(n, units):
        per = D // KU
        ks = pl.ds(blk(n % per, KU), units * KU)
        part = jnp.dot(pltpu.bitcast(xn_v[0:TB // 2, ks], bf16),
                       pltpu.bitcast(wp_v[pl.ds(blk(n, KU // 2), units * KU // 2), :], bf16),
                       preferred_element_type=f32)
        for j in range(NT):
            p = part[:, j * LANES:(j + 1) * LANES]
            dst = kvq0_v.at[n // per, j, PAD:PAD + TB, :]
            dst[...] = dst[...] + p

    def body_p(n, carry):
        wa_copy(n + 1).wait()
        k0_step(n, 1)
        permute_weight(n + 1, 1)
        return carry

    jax.lax.fori_loop(0, NU - 1, body_p, 0)
    x_copy(1).wait()
    k0_step(NU - 1, 1)
    do_ln(TB)
    k_v[:, TB:TB + PAD, :] = kvq0_v[0, :, TB:TB + PAD, :]
    v_v[:, TB:TB + PAD, :] = kvq0_v[1, :, TB:TB + PAD, :]

    def body_a(i, carry):
        x_copy(i + 1).wait()

        start = blk(i, TB)

        def att0():
            base0 = pl.multiple_of((i - 1) * 32, 32)
            plist = [(base0 + r, RA) for r in range(0, 32, RA)]
            plist.append((pl.multiple_of(jnp.minimum(TB - 32 + (i - 1) * 8, TB - 8), 8), 8))
            for tok0, rows in plist:

                def store(o, tok0=tok0, rows=rows):
                    o_v[pl.ds(pl.multiple_of(tok0, 8), rows), :] = o

                attention(kvq0_v.at[2], kvq0_v.at[0], kvq0_v.at[1], tok0, rows, True, store)

        project(0, k_v, start)
        project(1, v_v, start)
        project(2, q_v, start, Q_SCALE)
        att0()
        do_ln(start + TB)
        return carry

    jax.lax.fori_loop(1, NB, body_a, 0)

    for cp in w_copies:
        cp.wait()

    def body_b(i, carry):
        base = blk(i, TB)
        rows = pl.ds(base, TB)
        nbase = pl.multiple_of(jnp.minimum(i + 1, NB - 1) * TB, TB)
        oc_v[...] = o_v[...]
        nc = F // FC
        pieces = list(range(0, TB, RA))

        def att(rs):
            for r in rs:
                def store(o, r=r):
                    o_v[pl.ds(r, RA), :] = o
                attention(q_v, k_v, v_v, nbase + r, RA, False, store)

        acc = None
        for c in range(nc):
            sl = slice(c * FC, (c + 1) * FC)
            g = jnp.dot(xn_block(base), w1_v[:, sl], preferred_element_type=f32)
            u = jnp.dot(xn_block(base), w3_v[:, sl], preferred_element_type=f32)
            h = (_silu(g) * u).astype(bf16)
            d = jnp.dot(h, w2_v[sl, :], preferred_element_type=f32)
            acc = d if acc is None else acc + d
            att(pieces[(len(pieces) * c) // nc:(len(pieces) * (c + 1)) // nc])
        gate = _silu(acc)
        s = jnp.dot(oc_v[...], wo_v[...], preferred_element_type=f32)
        out_v[rows, :] = (x_v[rows, :].astype(f32) + s * gate).astype(bf16)
        out_copy(i).start()
        return carry

    jax.lax.fori_loop(0, NB, body_b, 0)
    for i in range(NB):
        out_copy(i).wait()


@jax.jit
def pallas_recurrent_scan__sliding_local_dilated__glu_gated_swiglu__prompt_kernel(
    A_x: jax.Array,
    A_wqkv: jax.Array,
    A_wo: jax.Array,
    B_x: jax.Array,
    B_w1: jax.Array,
    B_w3: jax.Array,
    B_w2: jax.Array,
):
    x = A_x.reshape(S, D)
    any_spec = pl.BlockSpec(memory_space=pl.ANY)
    out = pl.pallas_call(
        _kernel,
        out_shape=jax.ShapeDtypeStruct((S, D), bf16),
        in_specs=[any_spec] * 6,
        out_specs=any_spec,
        scratch_shapes=[
            pltpu.VMEM((S + TB, D), bf16),
            pltpu.VMEM(((S + TB) // 2, D), u32),
            pltpu.VMEM((3 * D, D), bf16),
            pltpu.VMEM((3 * D // 2, D), u32),
            pltpu.VMEM((D, D), bf16),
            pltpu.VMEM((D, F), bf16),
            pltpu.VMEM((D, F), bf16),
            pltpu.VMEM((F, D), bf16),
            pltpu.VMEM((3, NT, PAD + TB, LANES), f32),
            pltpu.VMEM((NT, PAD + S, LANES), f32),
            pltpu.VMEM((NT, PAD + S, LANES), f32),
            pltpu.VMEM((NT, PAD + S, LANES), f32),
            pltpu.VMEM((TB, D), bf16),
            pltpu.VMEM((TB, D), bf16),
            pltpu.VMEM((S, D), bf16),
            pltpu.SemaphoreType.DMA((NB + 1 + NU + 4,)),
            pltpu.SemaphoreType.DMA((NB,)),
        ],
        compiler_params=pltpu.CompilerParams(vmem_limit_bytes=120 * 1024 * 1024),
    )(x, A_wqkv, A_wo, B_w1, B_w3, B_w2)
    return out.reshape(1, S, D)
```

```python
import functools

import jax
import jax.numpy as jnp
from jax.experimental import pallas as pl
from jax.experimental.pallas import tpu as pltpu

S = 2048
D = 1024
F = 3584
H = 32
DH = D // H
W = 8
DIL = 2
PAD = 16
LANES = 128
NT = D // LANES
TB = 256
NB = S // TB
FC = 512
KU = 256
NU = 3 * D // KU
PR = 128
RA = 8
LNR = 32
EPS = 1e-5
MASK_VALUE = -1e9
Q_SCALE = DH ** -0.5 * 1.4426950408889634

f32 = jnp.float32
bf16 = jnp.bfloat16
u32 = jnp.uint32


def _swap_tile_lane_bits(tiles):
    lane = jax.lax.broadcasted_iota(jnp.int32, tiles[0].shape, 1)
    r = [tiles[0]] + [pltpu.roll(tiles[t], 4 * t, 1) for t in range(1, NT)]
    u = [r[(-k) % NT] for k in range(NT)]
    for b in range(3):
        m = (lane & (4 << b)) != 0
        u = [jnp.where(m, u[(k - (1 << b)) % NT], u[k]) for k in range(NT)]
    return [u[0]] + [pltpu.roll(u[t], LANES - 4 * t, 1) for t in range(1, NT)]


def _layernorm(x):
    x = x.astype(f32)
    m = jnp.mean(x, axis=-1, keepdims=True)
    xc = x - m
    v = jnp.mean(xc * xc, axis=-1, keepdims=True)
    return (xc * jax.lax.rsqrt(v + EPS)).astype(bf16)


def _silu(x):
    h = 0.5 * x
    return h + h * jnp.tanh(h)


def _kernel(x_hbm, wqkv_hbm, wo_hbm, w1_hbm, w3_hbm, w2_hbm, out_hbm,
            x_v, xn_v, wa_v, wp_v, wo_v, w1_v, w3_v, w2_v,
            kvq0_v, q_v, k_v, v_v, o_v, oc_v, out_v,
            in_sem, out_sem):

    X_SEM, WA_SEM, W_SEM = 0, NB + 1, NB + 1 + NU

    def blk(i, n):
        return i * n if isinstance(i, int) else pl.multiple_of(i * n, n)

    def x_copy(b):
        src = min(b, NB - 1) if isinstance(b, int) else jnp.minimum(b, NB - 1)
        return pltpu.make_async_copy(
            x_hbm.at[pl.ds(blk(src, TB), TB)], x_v.at[pl.ds(blk(b, TB), TB)], in_sem.at[X_SEM + b])

    def wa_copy(n):
        per = D // KU
        col = ((n // per + 1) % 3)
        return pltpu.make_async_copy(
            wqkv_hbm.at[pl.ds(blk(n % per, KU), KU), pl.ds(blk(col, D), D)],
            wa_v.at[pl.ds(blk(n, KU), KU)], in_sem.at[WA_SEM + n])

    w_copies = [
        pltpu.make_async_copy(w1_hbm, w1_v, in_sem.at[W_SEM + 0]),
        pltpu.make_async_copy(w3_hbm, w3_v, in_sem.at[W_SEM + 1]),
        pltpu.make_async_copy(w2_hbm, w2_v, in_sem.at[W_SEM + 2]),
        pltpu.make_async_copy(wo_hbm, wo_v, in_sem.at[W_SEM + 3]),
    ]

    def out_copy(i):
        rows = pl.ds(blk(i, TB), TB)
        return pltpu.make_async_copy(out_v.at[rows], out_hbm.at[rows], out_sem.at[i])

    def permute_weight(n, units):
        for r in range(0, units * KU, PR):
            rows = pl.ds(blk(n, KU) + r, PR)
            prows = pl.ds(blk(n, KU // 2) + r // 2, PR // 2)
            tiles = [pltpu.bitcast(wa_v[rows, j * LANES:(j + 1) * LANES], u32)
                     for j in range(NT)]
            tiles = _swap_tile_lane_bits(tiles)
            for j in range(NT):
                wp_v[prows, j * LANES:(j + 1) * LANES] = tiles[j]

    def half(start):
        return start // 2 if isinstance(start, int) else pl.multiple_of(start // 2, TB // 2)

    def do_ln(start):
        for r in range(0, TB, LNR):
            xn = _layernorm(x_v[pl.ds(start + r, LNR), :])
            xn_v[pl.ds(half(start) + r // 2, LNR // 2), :] = pltpu.bitcast(xn, u32)

    def xn_block(start):
        return pltpu.bitcast(xn_v[pl.ds(half(start), TB // 2), :], bf16)

    def project(sec, dst, start):
        w = pltpu.bitcast(wp_v[sec * D // 2:(sec + 1) * D // 2, :], bf16)
        res = jnp.dot(xn_block(start), w, preferred_element_type=f32)
        for j in range(NT):
            dst[j, pl.ds(PAD + start, TB), :] = res[:, j * LANES:(j + 1) * LANES]

    def attention(q_ref, k_ref, v_ref, tok0, rows, first_block, store):
        lane = jax.lax.broadcasted_iota(jnp.int32, (rows, LANES), 1)
        m1 = (lane & 1) != 0
        m2 = (lane & 2) != 0
        start = tok0 + PAD
        q = [q_ref[j, pl.ds(start, rows), :] * Q_SCALE for j in range(NT)]
        ls = []
        for w in range(W):
            acc = None
            for j in range(NT):
                p = q[j] * k_ref[j, pl.ds(start - DIL * w, rows), :]
                acc = p if acc is None else acc + p
            acc = acc + jnp.where(m1, pltpu.roll(acc, 1, 1), pltpu.roll(acc, LANES - 1, 1))
            acc = acc + jnp.where(m2, pltpu.roll(acc, 2, 1), pltpu.roll(acc, LANES - 2, 1))
            if first_block and w > 0:
                tok = jax.lax.broadcasted_iota(jnp.int32, (rows, LANES), 0) + tok0
                acc = jnp.where(tok >= DIL * w, acc, MASK_VALUE)
            ls.append(acc)
        mx = functools.reduce(jnp.maximum, ls)
        es = [jnp.exp2(l - mx) for l in ls]
        inv = 1.0 / functools.reduce(lambda a, b: a + b, es)
        ps = [e * inv for e in es]
        o = []
        for j in range(NT):
            acc = None
            for w in range(W):
                p = ps[w] * v_ref[j, pl.ds(start - DIL * w, rows), :]
                acc = p if acc is None else acc + p
            o.append(acc)
        o = _swap_tile_lane_bits(o)
        store(jnp.concatenate(o, axis=1).astype(bf16))

    x_copy(0).start()
    for n in range(NU):
        wa_copy(n).start()
    for b in range(1, NB + 1):
        x_copy(b).start()
    for cp in w_copies:
        cp.start()

    def zero_body(z, carry):
        kvq0_v[z] = jnp.zeros((NT, PAD + TB, LANES), f32)
        return carry

    jax.lax.fori_loop(0, 3, zero_body, 0)

    x_copy(0).wait()
    do_ln(0)
    wa_copy(0).wait()
    permute_weight(0, 1)

    def k0_step(n, units):
        per = D // KU
        ks = pl.ds(blk(n % per, KU), units * KU)
        part = jnp.dot(pltpu.bitcast(xn_v[0:TB // 2, ks], bf16),
                       pltpu.bitcast(wp_v[pl.ds(blk(n, KU // 2), units * KU // 2), :], bf16),
                       preferred_element_type=f32)
        for j in range(NT):
            p = part[:, j * LANES:(j + 1) * LANES]
            dst = kvq0_v.at[n // per, j, PAD:PAD + TB, :]
            dst[...] = dst[...] + p

    def body_p(n, carry):
        wa_copy(n + 1).wait()
        k0_step(n, 1)
        permute_weight(n + 1, 1)
        return carry

    jax.lax.fori_loop(0, NU - 1, body_p, 0)
    x_copy(1).wait()
    k0_step(NU - 1, 1)
    do_ln(TB)
    k_v[:, TB:TB + PAD, :] = kvq0_v[0, :, TB:TB + PAD, :]
    v_v[:, TB:TB + PAD, :] = kvq0_v[1, :, TB:TB + PAD, :]

    def body_a(i, carry):
        x_copy(i + 1).wait()

        start = blk(i, TB)

        base0 = pl.multiple_of((i - 1) * 32, 32)
        plist = [base0 + r for r in range(0, 32, RA)]
        plist.append(pl.multiple_of(jnp.minimum(TB - 32 + (i - 1) * 8, TB - 8), 8))

        def att0(p):
            tok0 = plist[p]

            def store(o):
                o_v[pl.ds(pl.multiple_of(tok0, 8), RA), :] = o

            attention(kvq0_v.at[2], kvq0_v.at[0], kvq0_v.at[1], tok0, RA, True, store)

        def ln1(p):
            r = p * LNR
            xn = _layernorm(x_v[pl.ds(start + TB + r, LNR), :])
            xn_v[pl.ds(half(start + TB) + r // 2, LNR // 2), :] = pltpu.bitcast(xn, u32)

        project(0, k_v, start)
        project(1, v_v, start)
        project(2, q_v, start)
        att0(0)
        att0(1)
        for p in range(4):
            ln1(p)
        att0(2)
        for p in range(4, 8):
            ln1(p)
        att0(3)
        att0(4)
        return carry

    jax.lax.fori_loop(1, NB, body_a, 0)

    for cp in w_copies:
        cp.wait()

    def body_b(i, carry):
        base = blk(i, TB)
        rows = pl.ds(base, TB)
        nbase = pl.multiple_of(jnp.minimum(i + 1, NB - 1) * TB, TB)
        oc_v[...] = o_v[...]
        nc = F // FC
        pieces = list(range(0, TB, RA))

        def att(rs):
            for r in rs:
                def store(o, r=r):
                    o_v[pl.ds(r, RA), :] = o
                attention(q_v, k_v, v_v, nbase + r, RA, False, store)

        acc = None
        for c in range(nc):
            sl = slice(c * FC, (c + 1) * FC)
            g = jnp.dot(xn_block(base), w1_v[:, sl], preferred_element_type=f32)
            u = jnp.dot(xn_block(base), w3_v[:, sl], preferred_element_type=f32)
            h = (_silu(g) * u).astype(bf16)
            d = jnp.dot(h, w2_v[sl, :], preferred_element_type=f32)
            acc = d if acc is None else acc + d
            att(pieces[(len(pieces) * c) // nc:(len(pieces) * (c + 1)) // nc])
        gate = _silu(acc)
        s = jnp.dot(oc_v[...], wo_v[...], preferred_element_type=f32)
        out_v[rows, :] = (x_v[rows, :].astype(f32) + s * gate).astype(bf16)
        out_copy(i).start()
        return carry

    jax.lax.fori_loop(0, NB, body_b, 0)
    for i in range(NB):
        out_copy(i).wait()


@jax.jit
def pallas_recurrent_scan__sliding_local_dilated__glu_gated_swiglu__prompt_kernel(
    A_x: jax.Array,
    A_wqkv: jax.Array,
    A_wo: jax.Array,
    B_x: jax.Array,
    B_w1: jax.Array,
    B_w3: jax.Array,
    B_w2: jax.Array,
):
    x = A_x.reshape(S, D)
    any_spec = pl.BlockSpec(memory_space=pl.ANY)
    out = pl.pallas_call(
        _kernel,
        out_shape=jax.ShapeDtypeStruct((S, D), bf16),
        in_specs=[any_spec] * 6,
        out_specs=any_spec,
        scratch_shapes=[
            pltpu.VMEM((S + TB, D), bf16),
            pltpu.VMEM(((S + TB) // 2, D), u32),
            pltpu.VMEM((3 * D, D), bf16),
            pltpu.VMEM((3 * D // 2, D), u32),
            pltpu.VMEM((D, D), bf16),
            pltpu.VMEM((D, F), bf16),
            pltpu.VMEM((D, F), bf16),
            pltpu.VMEM((F, D), bf16),
            pltpu.VMEM((3, NT, PAD + TB, LANES), f32),
            pltpu.VMEM((NT, PAD + S, LANES), f32),
            pltpu.VMEM((NT, PAD + S, LANES), f32),
            pltpu.VMEM((NT, PAD + S, LANES), f32),
            pltpu.VMEM((TB, D), bf16),
            pltpu.VMEM((TB, D), bf16),
            pltpu.VMEM((S, D), bf16),
            pltpu.SemaphoreType.DMA((NB + 1 + NU + 4,)),
            pltpu.SemaphoreType.DMA((NB,)),
        ],
        compiler_params=pltpu.CompilerParams(vmem_limit_bytes=120 * 1024 * 1024),
    )(x, A_wqkv, A_wo, B_w1, B_w3, B_w2)
    return out.reshape(1, S, D)
```

```python
import functools

import jax
import jax.numpy as jnp
from jax.experimental import pallas as pl
from jax.experimental.pallas import tpu as pltpu

S = 2048
D = 1024
F = 3584
H = 32
DH = D // H
W = 8
DIL = 2
PAD = 16
LANES = 128
NT = D // LANES
TB = 256
NB = S // TB
FC = 512
KU = 256
NU = 3 * D // KU
PR = 128
RA = 8
LNR = 32
EPS = 1e-5
MASK_VALUE = -1e9
Q_SCALE = DH ** -0.5 * 1.4426950408889634

f32 = jnp.float32
bf16 = jnp.bfloat16
u32 = jnp.uint32


def _swap_tile_lane_bits(tiles):
    lane = jax.lax.broadcasted_iota(jnp.int32, tiles[0].shape, 1)
    r = [tiles[0]] + [pltpu.roll(tiles[t], 4 * t, 1) for t in range(1, NT)]
    u = [r[(-k) % NT] for k in range(NT)]
    for b in range(3):
        m = (lane & (4 << b)) != 0
        u = [jnp.where(m, u[(k - (1 << b)) % NT], u[k]) for k in range(NT)]
    return [u[0]] + [pltpu.roll(u[t], LANES - 4 * t, 1) for t in range(1, NT)]


def _layernorm(x):
    x = x.astype(f32)
    m = jnp.mean(x, axis=-1, keepdims=True)
    xc = x - m
    v = jnp.mean(xc * xc, axis=-1, keepdims=True)
    return (xc * jax.lax.rsqrt(v + EPS)).astype(bf16)


def _silu(x):
    h = 0.5 * x
    return h + h * jnp.tanh(h)


def _kernel(x_hbm, wqkv_hbm, wo_hbm, w1_hbm, w3_hbm, w2_hbm, out_hbm,
            x_v, xn_v, wa_v, wp_v, wo_v, w1_v, w3_v, w2_v,
            kvq0_v, q_v, k_v, v_v, o_v, oc_v, out_v,
            in_sem, out_sem):

    X_SEM, WA_SEM, W_SEM = 0, NB + 1, NB + 1 + NU

    def blk(i, n):
        return i * n if isinstance(i, int) else pl.multiple_of(i * n, n)

    def x_copy(b):
        src = min(b, NB - 1) if isinstance(b, int) else jnp.minimum(b, NB - 1)
        return pltpu.make_async_copy(
            x_hbm.at[pl.ds(blk(src, TB), TB)], x_v.at[pl.ds(blk(b, TB), TB)], in_sem.at[X_SEM + b])

    def wa_copy(n):
        per = D // KU
        col = ((n // per + 1) % 3)
        return pltpu.make_async_copy(
            wqkv_hbm.at[pl.ds(blk(n % per, KU), KU), pl.ds(blk(col, D), D)],
            wa_v.at[pl.ds(blk(n, KU), KU)], in_sem.at[WA_SEM + n])

    w_copies = [
        pltpu.make_async_copy(w1_hbm, w1_v, in_sem.at[W_SEM + 0]),
        pltpu.make_async_copy(w3_hbm, w3_v, in_sem.at[W_SEM + 1]),
        pltpu.make_async_copy(w2_hbm, w2_v, in_sem.at[W_SEM + 2]),
        pltpu.make_async_copy(wo_hbm, wo_v, in_sem.at[W_SEM + 3]),
    ]

    def out_copy(i):
        rows = pl.ds(blk(i, TB), TB)
        return pltpu.make_async_copy(out_v.at[rows], out_hbm.at[rows], out_sem.at[i])

    def permute_weight(n, units):
        for r in range(0, units * KU, PR):
            rows = pl.ds(blk(n, KU) + r, PR)
            prows = pl.ds(blk(n, KU // 2) + r // 2, PR // 2)
            tiles = [pltpu.bitcast(wa_v[rows, j * LANES:(j + 1) * LANES], u32)
                     for j in range(NT)]
            tiles = _swap_tile_lane_bits(tiles)
            for j in range(NT):
                wp_v[prows, j * LANES:(j + 1) * LANES] = tiles[j]

    def half(start):
        return start // 2 if isinstance(start, int) else pl.multiple_of(start // 2, TB // 2)

    def do_ln(start):
        for r in range(0, TB, LNR):
            xn = _layernorm(x_v[pl.ds(start + r, LNR), :])
            xn_v[pl.ds(half(start) + r // 2, LNR // 2), :] = pltpu.bitcast(xn, u32)

    def xn_block(start):
        return pltpu.bitcast(xn_v[pl.ds(half(start), TB // 2), :], bf16)

    def project(sec, dst, start):
        w = pltpu.bitcast(wp_v[sec * D // 2:(sec + 1) * D // 2, :], bf16)
        res = jnp.dot(xn_block(start), w, preferred_element_type=f32)
        for j in range(NT):
            dst[j, pl.ds(PAD + start, TB), :] = res[:, j * LANES:(j + 1) * LANES]

    def attention(q_ref, k_ref, v_ref, tok0, rows, first_block, store):
        lane = jax.lax.broadcasted_iota(jnp.int32, (rows, LANES), 1)
        m1 = (lane & 1) != 0
        m2 = (lane & 2) != 0
        start = tok0 + PAD
        q = [q_ref[j, pl.ds(start, rows), :] * Q_SCALE for j in range(NT)]
        ls = []
        for w in range(W):
            acc = None
            for j in range(NT):
                p = q[j] * k_ref[j, pl.ds(start - DIL * w, rows), :]
                acc = p if acc is None else acc + p
            acc = acc + jnp.where(m1, pltpu.roll(acc, 1, 1), pltpu.roll(acc, LANES - 1, 1))
            acc = acc + jnp.where(m2, pltpu.roll(acc, 2, 1), pltpu.roll(acc, LANES - 2, 1))
            if first_block and w > 0:
                tok = jax.lax.broadcasted_iota(jnp.int32, (rows, LANES), 0) + tok0
                acc = jnp.where(tok >= DIL * w, acc, MASK_VALUE)
            ls.append(acc)
        mx = functools.reduce(jnp.maximum, ls)
        es = [jnp.exp2(l - mx) for l in ls]
        inv = 1.0 / functools.reduce(lambda a, b: a + b, es)
        ps = [e * inv for e in es]
        o = []
        for j in range(NT):
            acc = None
            for w in range(W):
                p = ps[w] * v_ref[j, pl.ds(start - DIL * w, rows), :]
                acc = p if acc is None else acc + p
            o.append(acc)
        o = _swap_tile_lane_bits(o)
        store(jnp.concatenate(o, axis=1).astype(bf16))

    x_copy(0).start()
    for n in range(NU):
        wa_copy(n).start()
    for b in range(1, NB + 1):
        x_copy(b).start()
    for cp in w_copies:
        cp.start()

    def zero_body(z, carry):
        kvq0_v[z] = jnp.zeros((NT, PAD + TB, LANES), f32)
        return carry

    jax.lax.fori_loop(0, 3, zero_body, 0)

    x_copy(0).wait()
    do_ln(0)
    wa_copy(0).wait()
    permute_weight(0, 1)

    def k0_step(n, units):
        per = D // KU
        ks = pl.ds(blk(n % per, KU), units * KU)
        part = jnp.dot(pltpu.bitcast(xn_v[0:TB // 2, ks], bf16),
                       pltpu.bitcast(wp_v[pl.ds(blk(n, KU // 2), units * KU // 2), :], bf16),
                       preferred_element_type=f32)
        for j in range(NT):
            p = part[:, j * LANES:(j + 1) * LANES]
            dst = kvq0_v.at[n // per, j, PAD:PAD + TB, :]
            dst[...] = dst[...] + p

    def body_p(n, carry):
        wa_copy(n + 1).wait()
        k0_step(n, 1)
        permute_weight(n + 1, 1)
        return carry

    jax.lax.fori_loop(0, NU - 1, body_p, 0)
    x_copy(1).wait()
    k0_step(NU - 1, 1)
    do_ln(TB)
    k_v[:, TB:TB + PAD, :] = kvq0_v[0, :, TB:TB + PAD, :]
    v_v[:, TB:TB + PAD, :] = kvq0_v[1, :, TB:TB + PAD, :]

    def body_a(i, carry):
        x_copy(i + 1).wait()

        start = blk(i, TB)

        base0 = pl.multiple_of(jnp.minimum((i - 1) * 64, TB - 64), 64)
        plist = [base0 + r for r in range(0, 64, RA)]

        def att0(p):
            tok0 = plist[p]

            def store(o):
                o_v[pl.ds(pl.multiple_of(tok0, 8), RA), :] = o

            attention(kvq0_v.at[2], kvq0_v.at[0], kvq0_v.at[1], tok0, RA, True, store)

        def ln1(p):
            r = p * LNR
            xn = _layernorm(x_v[pl.ds(start + TB + r, LNR), :])
            xn_v[pl.ds(half(start + TB) + r // 2, LNR // 2), :] = pltpu.bitcast(xn, u32)

        project(0, k_v, start)
        project(1, v_v, start)
        project(2, q_v, start)
        for tok in 'a0 a1 a2 a3 a4 l0 l1 l2 l3 a5 l4 l5 l6 l7 a6 a7'.split():
            (att0 if tok[0] == 'a' else ln1)(int(tok[1:]))
        return carry

    jax.lax.fori_loop(1, NB, body_a, 0)

    for cp in w_copies:
        cp.wait()

    def body_b(i, carry):
        base = blk(i, TB)
        rows = pl.ds(base, TB)
        nbase = pl.multiple_of(jnp.minimum(i + 1, NB - 1) * TB, TB)
        oc_v[...] = o_v[...]
        nc = F // FC
        pieces = list(range(0, TB, RA))

        def att(rs):
            for r in rs:
                def store(o, r=r):
                    o_v[pl.ds(r, RA), :] = o
                attention(q_v, k_v, v_v, nbase + r, RA, False, store)

        acc = None
        for c in range(nc):
            sl = slice(c * FC, (c + 1) * FC)
            g = jnp.dot(xn_block(base), w1_v[:, sl], preferred_element_type=f32)
            u = jnp.dot(xn_block(base), w3_v[:, sl], preferred_element_type=f32)
            h = (_silu(g) * u).astype(bf16)
            d = jnp.dot(h, w2_v[sl, :], preferred_element_type=f32)
            acc = d if acc is None else acc + d
            att(pieces[(len(pieces) * c) // nc:(len(pieces) * (c + 1)) // nc])
        gate = _silu(acc)
        s = jnp.dot(oc_v[...], wo_v[...], preferred_element_type=f32)
        out_v[rows, :] = (x_v[rows, :].astype(f32) + s * gate).astype(bf16)
        out_copy(i).start()
        return carry

    jax.lax.fori_loop(0, NB, body_b, 0)
    for i in range(NB):
        out_copy(i).wait()


@jax.jit
def pallas_recurrent_scan__sliding_local_dilated__glu_gated_swiglu__prompt_kernel(
    A_x: jax.Array,
    A_wqkv: jax.Array,
    A_wo: jax.Array,
    B_x: jax.Array,
    B_w1: jax.Array,
    B_w3: jax.Array,
    B_w2: jax.Array,
):
    x = A_x.reshape(S, D)
    any_spec = pl.BlockSpec(memory_space=pl.ANY)
    out = pl.pallas_call(
        _kernel,
        out_shape=jax.ShapeDtypeStruct((S, D), bf16),
        in_specs=[any_spec] * 6,
        out_specs=any_spec,
        scratch_shapes=[
            pltpu.VMEM((S + TB, D), bf16),
            pltpu.VMEM(((S + TB) // 2, D), u32),
            pltpu.VMEM((3 * D, D), bf16),
            pltpu.VMEM((3 * D // 2, D), u32),
            pltpu.VMEM((D, D), bf16),
            pltpu.VMEM((D, F), bf16),
            pltpu.VMEM((D, F), bf16),
            pltpu.VMEM((F, D), bf16),
            pltpu.VMEM((3, NT, PAD + TB, LANES), f32),
            pltpu.VMEM((NT, PAD + S, LANES), f32),
            pltpu.VMEM((NT, PAD + S, LANES), f32),
            pltpu.VMEM((NT, PAD + S, LANES), f32),
            pltpu.VMEM((TB, D), bf16),
            pltpu.VMEM((TB, D), bf16),
            pltpu.VMEM((S, D), bf16),
            pltpu.SemaphoreType.DMA((NB + 1 + NU + 4,)),
            pltpu.SemaphoreType.DMA((NB,)),
        ],
        compiler_params=pltpu.CompilerParams(vmem_limit_bytes=120 * 1024 * 1024),
    )(x, A_wqkv, A_wo, B_w1, B_w3, B_w2)
    return out.reshape(1, S, D)
```
